```python
import os as _os
_os.environ.setdefault("JAX_PLATFORMS", "cpu")
import jax
import jax.numpy as jnp

def _softmax(x, axis=-1):
    return jax.nn.softmax(x, axis=axis)
def _gelu(x):
    return jax.nn.gelu(x, approximate=True)
def _silu(x):
    return jax.nn.silu(x)
def _sigmoid(x):
    return jax.nn.sigmoid(x)
def _layernorm(x, axis=-1, eps=1e-5):
    m = jnp.mean(x, axis=axis, keepdims=True)
    v = jnp.var(x, axis=axis, keepdims=True)
    return (x - m) / jnp.sqrt(v + eps)
def _scatter_add(tgt, idx, src, axis=0):
    return tgt.at[idx].add(src)
def _segment_sum(src, seg, n):
    return jax.ops.segment_sum(src, seg, n)
class _Rng:
    def __init__(self, key):
        self._k = key
    def _next(self):
        self._k, sub = jax.random.split(self._k)
        return sub
    def normal(self, shape):
        return jax.random.normal(self._next(), shape, dtype=jnp.bfloat16)
    def randint(self, lo, hi, shape):
        return jax.random.randint(self._next(), shape, lo, hi, dtype=jnp.int32)
    def uniform(self, shape, lo=0.0, hi=1.0):
        return jax.random.uniform(self._next(), shape, jnp.bfloat16, lo, hi)
    def permutation(self, n):
        return jax.random.permutation(self._next(), n)


kernel_name = 'standalone__gqa_softmax__decode'

def setup_inputs():
    _rng = _Rng(jax.random.key(int.from_bytes(__import__("os").urandom(4), "little")))
    _w = (lambda a: (lambda t: t.astype(jnp.bfloat16) if jnp.issubdtype(t.dtype, jnp.floating) else t)(jnp.asarray(a)))
    B, Hq, Hkv, Sq, Sk, D = 2, 32, 32, 1, 8192, 128
    return {
        "q": _w((lambda *s: _rng.normal(s) * 0.8)(B, Hq, Sq, D)),
        "k": _w((lambda *s: _rng.normal(s) * 0.8)(B, Hkv, Sk, D)),
        "v": _w((lambda *s: _rng.normal(s) * 0.05)(B, Hkv, Sk, D)),
    }

def reference(q, k, v):
    B, Hq, Sq, D = q.shape
    Hkv = k.shape[1]
    rep = Hq // Hkv
    k = jnp.repeat(k, rep, axis=1)
    v = jnp.repeat(v, rep, axis=1)
    scale = D ** -0.5
    scores = jnp.einsum("bhqd,bhkd->bhqk", q, k) * scale
    p = _softmax(scores, axis=-1)
    return jnp.einsum("bhqk,bhkd->bhqd", p, v)
```

```python
import jax
import jax.numpy as jnp
from jax import lax
import jax.experimental.pallas as pl
import jax.experimental.pallas.tpu as pltpu


@jax.jit
def pallas_standalone__gqa_softmax__decode_kernel(
    q: jax.Array,
    k: jax.Array,
    v: jax.Array,
):
    Bq, Hq, Sq, Dd = q.shape
    Hkv, Sk = k.shape[1], k.shape[2]
    assert Sq == 1 and Hq == Hkv
    BH = Bq * Hq
    G = 8
    GHI = 1
    R = 128
    r = 16
    NB = 6
    LAG = NB - 1
    GLO = G - GHI
    A = BH // G
    nper = Sk // R
    n = A * nper
    nsteps = R // r
    scale = Dd ** -0.5

    q2 = q.reshape(BH, Dd)
    k4 = k.reshape(A, G, Sk, Dd)
    v4 = v.reshape(A, G, Sk, Dd)

    def kern(q_hbm, k_hbm, v_hbm, o_ref, qbuf, kbuf, vbuf, qsem, ksem, vsem,
             m_sc, l_sc, acc_sc, out_sc):
        def desc(which, hi, a, row0, slot, t):
            src, buf, sem = (k_hbm, kbuf, ksem) if which == 0 else (v_hbm, vbuf, vsem)
            g0, gn = (GLO, GHI) if hi else (0, GLO)
            rows = pl.ds(pl.multiple_of(row0 + t * r, r), r)
            return pltpu.make_async_copy(
                src.at[a, pl.ds(g0, gn), rows, :],
                buf.at[slot, pl.ds(g0, gn), pl.ds(t * r, r), :],
                sem.at[slot])

        def issue_half(a, row0, slot, hs):
            t = hs // 2
            w = hs % 2
            desc(w, True, a, row0, slot, t).start(priority=0)
            desc(1 - w, False, a, row0, slot, t).start(priority=1)

        def wait(slot):
            pltpu.make_async_copy(kbuf.at[slot], kbuf.at[slot], ksem.at[slot]).wait()
            pltpu.make_async_copy(vbuf.at[slot], vbuf.at[slot], vsem.at[slot]).wait()

        qcp = pltpu.make_async_copy(q_hbm, qbuf, qsem.at[0])
        qcp.start()
        for j in range(LAG):
            for hs in range(2 * nsteps):
                issue_half(j // nper, (j % nper) * R, j, hs)
        qcp.wait()
        row = lax.broadcasted_iota(jnp.int32, (G, Dd), 0)
        rowR = lax.broadcasted_iota(jnp.int32, (G, R), 0)

        def batch(i, do_issue):
            a = i // nper
            c = i % nper
            slot = i % NB
            j = i + LAG
            ja = j // nper
            jrow = (j % nper) * R
            jslot = j % NB
            wait(slot)
            nh = 2 * nsteps
            st = {}
            q8 = qbuf[pl.ds(pl.multiple_of(a * G, G), G), :]
            first = c == 0

            def qk(gs):
                def fn():
                    for g in gs:
                        sg = lax.dot_general(
                            q8, kbuf[slot, g], (((1,), (1,)), ((), ())),
                            preferred_element_type=jnp.float32)
                        st['s'] = sg if 's' not in st else jnp.where(rowR == g, sg, st['s'])
                return fn

            def sm():
                s = st['s'] * scale
                m_old = jnp.where(first, -jnp.inf, m_sc[...])
                m_new = jnp.maximum(m_old, jnp.max(s, axis=-1, keepdims=True))
                alpha = jnp.exp(m_old - m_new)
                p = jnp.exp(s - m_new[:, 0:1])
                psum = p[:, 0:Dd]
                for u in range(1, R // Dd):
                    psum = psum + p[:, u * Dd:(u + 1) * Dd]
                l_old = jnp.where(first, 0.0, l_sc[...])
                l_sc[...] = l_old * alpha + psum
                m_sc[...] = m_new
                st['p'] = p.astype(jnp.bfloat16)
                st['alpha'] = alpha

            def pv(gs):
                def fn():
                    for g in gs:
                        og = jnp.dot(st['p'], vbuf[slot, g],
                                     preferred_element_type=jnp.float32)
                        st['o'] = og if 'o' not in st else jnp.where(row == g, og, st['o'])
                return fn

            def upd():
                acc_old = jnp.where(first, 0.0, acc_sc[...])
                acc_sc[...] = acc_old * st['alpha'] + st['o']

            half = G // 2
            pieces = [qk(range(0, half)), qk(range(half, G)), sm,
                      pv(range(0, half)), pv(range(half, G)), upd]
            for hs in range(nh):
                if do_issue:
                    issue_half(ja, jrow, jslot, hs)
                lo = hs * len(pieces) // nh
                hi = (hs + 1) * len(pieces) // nh
                for pc in pieces[lo:hi]:
                    pc()

            @pl.when(c == nper - 1)
            def _():
                l = jnp.sum(l_sc[...], axis=-1, keepdims=True)
                out_sc[pl.ds(pl.multiple_of(a * G, G), G), :] = acc_sc[...] / l

        m_sc[...] = jnp.zeros_like(m_sc)
        l_sc[...] = jnp.ones_like(l_sc)
        acc_sc[...] = jnp.zeros_like(acc_sc)

        def body1(i, c):
            batch(i, True)
            return c

        def body2(i, c):
            batch(i, False)
            return c

        lax.fori_loop(0, n - LAG, body1, 0)
        lax.fori_loop(n - LAG, n, body2, 0)
        o_ref[...] = out_sc[...].astype(o_ref.dtype)

    out = pl.pallas_call(
        kern,
        in_specs=[pl.BlockSpec(memory_space=pl.ANY)] * 3,
        out_specs=pl.BlockSpec(memory_space=pltpu.VMEM),
        out_shape=jax.ShapeDtypeStruct((BH, Dd), q.dtype),
        scratch_shapes=[
            pltpu.VMEM((BH, Dd), q.dtype),
            pltpu.VMEM((NB, G, R, Dd), k.dtype),
            pltpu.VMEM((NB, G, R, Dd), v.dtype),
            pltpu.SemaphoreType.DMA((1,)),
            pltpu.SemaphoreType.DMA((NB,)),
            pltpu.SemaphoreType.DMA((NB,)),
            pltpu.VMEM((G, Dd), jnp.float32),
            pltpu.VMEM((G, Dd), jnp.float32),
            pltpu.VMEM((G, Dd), jnp.float32),
            pltpu.VMEM((BH, Dd), jnp.float32),
        ],
        compiler_params=pltpu.CompilerParams(
            vmem_limit_bytes=64 * 1024 * 1024, disable_bounds_checks=True),
    )(q2, k4, v4)
    return out.reshape(Bq, Hq, Sq, Dd)
```

```python
import jax
import jax.numpy as jnp
from jax import lax
import jax.experimental.pallas as pl
import jax.experimental.pallas.tpu as pltpu

_G = 8
_U = 2
_R = 128
_RP = 16
_NHI = 2
_NB = 8
_LAG = 7


def _compiler_params():
    try:
        return pltpu.CompilerParams(disable_semaphore_checks=True)
    except TypeError:
        return pltpu.CompilerParams()


@jax.jit
def pallas_standalone__gqa_softmax__decode_kernel(
    q: jax.Array,
    k: jax.Array,
    v: jax.Array,
):
    B, Hq, Sq, D = q.shape
    Hkv, Sk = k.shape[1], k.shape[2]
    assert Sq == 1 and Hq == Hkv, "decode shape with one KV head per query head"
    G, U, R, RP, NHI, NB, LAG = _G, _U, _R, _RP, _NHI, _NB, _LAG
    BH = B * Hq
    A = BH // G
    NS = G * U
    NLO = NS - NHI
    L = Sk // U
    nper = L // R
    T = R // RP
    assert BH % G == 0 and Sk % (U * R) == 0 and R % D == 0
    assert nper % NB == 0 and LAG < NB and LAG < nper
    scale = D ** -0.5

    q2 = q.reshape(BH, D)
    k4 = k.reshape(A, NS, L, D)
    v4 = v.reshape(A, NS, L, D)

    def kernel(q_hbm, k_hbm, v_hbm, o_ref, qbuf, buf, qsem, sem, s_sc, out_sc):
        def issue(src, a, c, t):
            slot = c % NB
            rows = pl.ds(pl.multiple_of(c * R + t * RP, RP), RP)
            for s0, sn, prio in ((NLO, NHI, 0), (0, NLO, 1)):
                pltpu.make_async_copy(
                    src.at[a, pl.ds(s0, sn), rows, :],
                    buf.at[slot, pl.ds(s0, sn), pl.ds(t * RP, RP), :],
                    sem.at[slot],
                ).start(priority=prio)

        def wait(slot):
            pltpu.make_async_copy(buf.at[slot], buf.at[slot], sem.at[slot]).wait()

        q_copy = pltpu.make_async_copy(q_hbm, qbuf, qsem.at[0])
        for j in range(LAG):
            for t in range(T):
                issue(k_hbm, 0, j, t)
            if j == 0:
                q_copy.start()
        q_copy.wait()

        row_d = lax.broadcasted_iota(jnp.int32, (G, D), 0)
        row_r = lax.broadcasted_iota(jnp.int32, (G, R), 0)

        def interleave(tile, order, nxt):
            for t in range(T):
                if nxt is not None:
                    issue(*nxt, t)
                for s in order[t * NS // T:(t + 1) * NS // T]:
                    tile(s)

        def k_batch(q8, c, mx, nxt):
            slot = c % NB
            wait(slot)
            sc = [None] * U

            def tile(s):
                g, u = divmod(s, U)
                sg = lax.dot_general(
                    q8, buf[slot, s], (((1,), (1,)), ((), ())),
                    preferred_element_type=jnp.float32)
                sc[u] = sg if sc[u] is None else jnp.where(row_r == g, sg, sc[u])

            interleave(tile, [g * U + u for u in range(U) for g in range(G)], nxt)
            for u in range(U):
                s = sc[u] * scale
                s_sc[u, c] = s
                for w in range(R // D):
                    mx = jnp.maximum(mx, s[:, w * D:(w + 1) * D])
            return mx

        def v_batch(m, c, carry, nxt):
            l, acc = carry
            slot = c % NB
            ps = []
            for u in range(U):
                p = jnp.exp(s_sc[u, c] - m)
                for w in range(R // D):
                    l = l + p[:, w * D:(w + 1) * D]
                ps.append(p.astype(v_hbm.dtype))
            wait(slot)
            st = {}

            def tile(s):
                g, u = divmod(s, U)
                og = jnp.dot(ps[u], buf[slot, s], preferred_element_type=jnp.float32)
                og = og if u == 0 else og + st["head"]
                if u < U - 1:
                    st["head"] = og
                else:
                    st["out"] = og if g == 0 else jnp.where(row_d == g, og, st["out"])

            interleave(tile, list(range(NS)), nxt)
            return l, acc + st["out"]

        def group(a, last):
            rows = pl.ds(pl.multiple_of(a * G, G), G)
            q8 = qbuf[rows, :]
            mx = jnp.full((G, D), -jnp.inf, jnp.float32)
            mx = lax.fori_loop(
                0, nper - LAG,
                lambda c, mx: k_batch(q8, c, mx, (k_hbm, a, c + LAG)), mx)
            mx = lax.fori_loop(
                nper - LAG, nper,
                lambda c, mx: k_batch(q8, c, mx, (v_hbm, a, c + LAG - nper)), mx)
            m = jnp.max(mx, axis=-1, keepdims=True)
            carry = (jnp.zeros((G, D), jnp.float32), jnp.zeros((G, D), jnp.float32))
            carry = lax.fori_loop(
                0, nper - LAG,
                lambda c, cr: v_batch(m, c, cr, (v_hbm, a, c + LAG)), carry)
            carry = lax.fori_loop(
                nper - LAG, nper,
                lambda c, cr: v_batch(
                    m, c, cr, None if last else (k_hbm, a + 1, c + LAG - nper)),
                carry)
            l, acc = carry
            out_sc[rows, :] = acc / jnp.sum(l, axis=-1, keepdims=True)

        def group_body(a, carry):
            group(a, False)
            return carry

        lax.fori_loop(0, A - 1, group_body, 0)
        group(A - 1, True)
        o_ref[...] = out_sc[...].astype(o_ref.dtype)

    out = pl.pallas_call(
        kernel,
        in_specs=[pl.BlockSpec(memory_space=pl.ANY)] * 3,
        out_specs=pl.BlockSpec(memory_space=pltpu.VMEM),
        out_shape=jax.ShapeDtypeStruct((BH, D), q.dtype),
        scratch_shapes=[
            pltpu.VMEM((BH, D), q.dtype),
            pltpu.VMEM((NB, NS, R, D), k.dtype),
            pltpu.SemaphoreType.DMA((1,)),
            pltpu.SemaphoreType.DMA((NB,)),
            pltpu.VMEM((U, nper, G, R), jnp.float32),
            pltpu.VMEM((BH, D), jnp.float32),
        ],
        compiler_params=_compiler_params(),
    )(q2, k4, v4)
    return out.reshape(B, Hq, Sq, D)
```

```python
import jax
import jax.numpy as jnp
from jax import lax
import jax.experimental.pallas as pl
import jax.experimental.pallas.tpu as pltpu

_G = 8
_U = 2
_R = 128
_RP = 16
_NHI = 2
_NB = 8
_LAG = 7


def _compiler_params():
    try:
        return pltpu.CompilerParams(disable_semaphore_checks=True)
    except TypeError:
        return pltpu.CompilerParams()


@jax.jit
def pallas_standalone__gqa_softmax__decode_kernel(
    q: jax.Array,
    k: jax.Array,
    v: jax.Array,
):
    B, Hq, Sq, D = q.shape
    Hkv, Sk = k.shape[1], k.shape[2]
    assert Sq == 1 and Hq == Hkv, "decode shape with one KV head per query head"
    G, U, R, RP, NHI, NB, LAG = _G, _U, _R, _RP, _NHI, _NB, _LAG
    BH = B * Hq
    A = BH // G
    NS = G * U
    NLO = NS - NHI
    L = Sk // U
    nper = L // R
    T = R // RP
    assert BH % G == 0 and Sk % (U * R) == 0 and R % D == 0
    assert nper % NB == 0 and LAG < NB and LAG < nper
    scale = D ** -0.5

    q3 = q.reshape(A, G, D)
    k4 = k.reshape(A, NS, L, D)
    v4 = v.reshape(A, NS, L, D)

    def kernel(q_hbm, k_hbm, v_hbm, o_ref, qbuf, buf, qsem, sem, s_sc, out_sc):
        def issue(src, a, c, t):
            slot = c % NB
            rows = pl.ds(pl.multiple_of(c * R + t * RP, RP), RP)
            for s0, sn, prio in ((NLO, NHI, 0), (0, NLO, 1)):
                pltpu.make_async_copy(
                    src.at[a, pl.ds(s0, sn), rows, :],
                    buf.at[slot, pl.ds(s0, sn), pl.ds(t * RP, RP), :],
                    sem.at[slot],
                ).start(priority=prio)

        def wait(slot):
            pltpu.make_async_copy(buf.at[slot], buf.at[slot], sem.at[slot]).wait()

        q_copy = pltpu.make_async_copy(q_hbm, qbuf, qsem.at[0])
        for j in range(LAG):
            for t in range(T):
                issue(k_hbm, 0, j, t)
            if j == 0:
                q_copy.start()
        q_copy.wait()

        row_d = lax.broadcasted_iota(jnp.int32, (G, D), 0)
        row_r = lax.broadcasted_iota(jnp.int32, (G, R), 0)

        def interleave(tile, order, nxt):
            for t in range(T):
                if nxt is not None:
                    issue(*nxt, t)
                for s in order[t * NS // T:(t + 1) * NS // T]:
                    tile(s)

        def k_batch(q8, c, mx, nxt):
            slot = c % NB
            wait(slot)
            sc = [None] * U

            def tile(s):
                g, u = divmod(s, U)
                sg = lax.dot_general(
                    q8, buf[slot, s], (((1,), (1,)), ((), ())),
                    preferred_element_type=jnp.float32)
                sc[u] = sg if sc[u] is None else jnp.where(row_r == g, sg, sc[u])

            interleave(tile, [g * U + u for u in range(U) for g in range(G)], nxt)
            for u in range(U):
                s = sc[u] * scale
                s_sc[u, c] = s
                for w in range(R // D):
                    mx = jnp.maximum(mx, s[:, w * D:(w + 1) * D])
            return mx

        def v_batch(m, c, carry, nxt):
            l, acc = carry
            slot = c % NB
            ps = []
            for u in range(U):
                p = jnp.exp(s_sc[u, c] - m)
                for w in range(R // D):
                    l = l + p[:, w * D:(w + 1) * D]
                ps.append(p.astype(v_hbm.dtype))
            wait(slot)
            st = {}

            def tile(s):
                g, u = divmod(s, U)
                og = jnp.dot(ps[u], buf[slot, s], preferred_element_type=jnp.float32)
                og = og if u == 0 else og + st["head"]
                if u < U - 1:
                    st["head"] = og
                else:
                    st["out"] = og if g == 0 else jnp.where(row_d == g, og, st["out"])

            interleave(tile, list(range(NS)), nxt)
            return l, acc + st["out"]

        def group(a, last):
            q8 = qbuf[a]
            mx = jnp.full((G, D), -jnp.inf, jnp.float32)
            mx = lax.fori_loop(
                0, nper - LAG,
                lambda c, mx: k_batch(q8, c, mx, (k_hbm, a, c + LAG)), mx)
            mx = lax.fori_loop(
                nper - LAG, nper,
                lambda c, mx: k_batch(q8, c, mx, (v_hbm, a, c + LAG - nper)), mx)
            m = jnp.max(mx, axis=-1, keepdims=True)
            carry = (jnp.zeros((G, D), jnp.float32), jnp.zeros((G, D), jnp.float32))
            carry = lax.fori_loop(
                0, nper - LAG,
                lambda c, cr: v_batch(m, c, cr, (v_hbm, a, c + LAG)), carry)
            carry = lax.fori_loop(
                nper - LAG, nper,
                lambda c, cr: v_batch(
                    m, c, cr, None if last else (k_hbm, a + 1, c + LAG - nper)),
                carry)
            l, acc = carry
            rows = pl.ds(pl.multiple_of(a * G, G), G)
            out_sc[rows, :] = acc / jnp.sum(l, axis=-1, keepdims=True)

        def group_body(a, carry):
            group(a, False)
            return carry

        lax.fori_loop(0, A - 1, group_body, 0)
        group(A - 1, True)
        o_ref[...] = out_sc[...].astype(o_ref.dtype)

    out = pl.pallas_call(
        kernel,
        in_specs=[pl.BlockSpec(memory_space=pl.ANY)] * 3,
        out_specs=pl.BlockSpec(memory_space=pltpu.VMEM),
        out_shape=jax.ShapeDtypeStruct((BH, D), q.dtype),
        scratch_shapes=[
            pltpu.VMEM((A, G, D), q.dtype),
            pltpu.VMEM((NB, NS, R, D), k.dtype),
            pltpu.SemaphoreType.DMA((1,)),
            pltpu.SemaphoreType.DMA((NB,)),
            pltpu.VMEM((U, nper, G, R), jnp.float32),
            pltpu.VMEM((BH, D), jnp.float32),
        ],
        compiler_params=_compiler_params(),
    )(q3, k4, v4)
    return out.reshape(B, Hq, Sq, D)
```

```python
import jax
import jax.numpy as jnp
from jax import lax
import jax.experimental.pallas as pl
import jax.experimental.pallas.tpu as pltpu

_G = 8
_U = 4
_R = 128
_TR = 8
_HI_FRAC = 8
_NB = 8
_LAG = 5
_PARTS = (16, 8, 8)


def _compiler_params():
    try:
        return pltpu.CompilerParams(disable_semaphore_checks=True)
    except TypeError:
        return pltpu.CompilerParams()


@jax.jit
def pallas_standalone__gqa_softmax__decode_kernel(
    q: jax.Array,
    k: jax.Array,
    v: jax.Array,
):
    B, Hq, Sq, D = q.shape
    Hkv, Sk = k.shape[1], k.shape[2]
    assert Sq == 1 and Hq == Hkv, "decode shape with one KV head per query head"
    G, U, R, TR, NB, LAG, PARTS = _G, _U, _R, _TR, _NB, _LAG, _PARTS
    BH = B * Hq
    A = BH // G
    NS = G * U
    L = Sk // U
    nper = L // R
    T = R // TR
    assert BH % G == 0 and Sk % (U * R) == 0 and R % D == 0 and NS % T == 0
    assert nper % NB == 0 and LAG < NB and LAG < nper and sum(PARTS) == NS
    part_start = [sum(PARTS[:j]) for j in range(len(PARTS))]
    scale = D ** -0.5

    q3 = q.reshape(A, G, D)
    k5 = k.reshape(A, NS, L // TR, TR, D)
    v5 = v.reshape(A, NS, L // TR, TR, D)

    def kernel(q_hbm, k_hbm, v_hbm, o_ref,
               qbuf, buf, qsem, sem, last_sem, s_sc, out_sc):
        def start_copies(src, a, c, t, s0, sn, dma_sem):
            n_hi = sn // _HI_FRAC
            for lo, n, prio in ((s0 + sn - n_hi, n_hi, 0), (s0, sn - n_hi, 1)):
                pltpu.make_async_copy(
                    src.at[a, pl.ds(lo, n), pl.ds(c * T + t, 1)],
                    buf.at[c % NB, pl.ds(lo, n), pl.ds(t, 1)],
                    dma_sem,
                ).start(priority=prio)

        def issue(src, a, c, t):
            start_copies(src, a, c, t, 0, NS, sem.at[c % NB])

        def issue_last(src, a, c, t):
            for i in range(t * len(PARTS), (t + 1) * len(PARTS)):
                j, tt = divmod(i, T)
                start_copies(src, a, c, tt, part_start[j], PARTS[j], last_sem.at[j])

        def wait(view, dma_sem):
            pltpu.make_async_copy(view, view, dma_sem).wait()

        q_copy = pltpu.make_async_copy(q_hbm, qbuf, qsem.at[0])
        for j in range(LAG):
            for t in range(T):
                issue(k_hbm, 0, j, t)
            if j == 0:
                q_copy.start()
        q_copy.wait()

        row_d = lax.broadcasted_iota(jnp.int32, (G, D), 0)
        row_r = lax.broadcasted_iota(jnp.int32, (G, R), 0)

        def interleave(tile, order, nxt):
            for t in range(T):
                if nxt is not None:
                    nxt(t)
                for s in order[t * NS // T:(t + 1) * NS // T]:
                    tile(s)

        def k_batch(q8, c, mx, nxt):
            slot = c % NB
            wait(buf.at[slot], sem.at[slot])
            sc = [None] * U

            def tile(s):
                g, u = divmod(s, U)
                sg = lax.dot_general(
                    q8, buf[slot, s].reshape(R, D), (((1,), (1,)), ((), ())),
                    preferred_element_type=jnp.float32)
                sc[u] = sg if g == 0 else jnp.where(row_r == g, sg, sc[u])

            interleave(tile, [g * U + u for u in range(U) for g in range(G)], nxt)
            for u in range(U):
                s = sc[u] * scale
                s_sc[u, c] = s
                for w in range(R // D):
                    mx = jnp.maximum(mx, s[:, w * D:(w + 1) * D])
            return mx

        def v_batch(m, c, carry, nxt, in_parts=False):
            l, acc = carry
            slot = c % NB
            ps = []
            for u in range(U):
                p = jnp.exp(s_sc[u, c] - m)
                for w in range(R // D):
                    l = l + p[:, w * D:(w + 1) * D]
                ps.append(p.astype(v_hbm.dtype))
            if not in_parts:
                wait(buf.at[slot], sem.at[slot])
            st = {}

            def tile(s):
                g, u = divmod(s, U)
                if in_parts and s in part_start:
                    j = part_start.index(s)
                    wait(buf.at[slot, pl.ds(s, PARTS[j])], last_sem.at[j])
                og = jnp.dot(ps[u], buf[slot, s].reshape(R, D),
                             preferred_element_type=jnp.float32)
                og = og if u == 0 else og + st["head"]
                if u < U - 1:
                    st["head"] = og
                else:
                    st["out"] = og if g == 0 else jnp.where(row_d == g, og, st["out"])

            interleave(tile, list(range(NS)), nxt)
            return l, acc + st["out"]

        def group(a, last):
            q8 = qbuf[a]
            mx = jnp.full((G, D), -jnp.inf, jnp.float32)
            mx = lax.fori_loop(
                0, nper - LAG,
                lambda c, mx: k_batch(
                    q8, c, mx, lambda t: issue(k_hbm, a, c + LAG, t)), mx)
            mx = lax.fori_loop(
                nper - LAG, nper,
                lambda c, mx: k_batch(
                    q8, c, mx, lambda t: issue(v_hbm, a, c + LAG - nper, t)), mx)
            m = jnp.max(mx, axis=-1, keepdims=True)
            carry = (jnp.zeros((G, D), jnp.float32), jnp.zeros((G, D), jnp.float32))
            carry = lax.fori_loop(
                0, nper - LAG - (1 if last else 0),
                lambda c, cr: v_batch(
                    m, c, cr, lambda t: issue(v_hbm, a, c + LAG, t)), carry)
            if last:
                carry = v_batch(m, nper - LAG - 1, carry,
                                lambda t: issue_last(v_hbm, a, nper - 1, t))
                carry = lax.fori_loop(
                    nper - LAG, nper - 1,
                    lambda c, cr: v_batch(m, c, cr, None), carry)
                carry = v_batch(m, nper - 1, carry, None, in_parts=True)
            else:
                carry = lax.fori_loop(
                    nper - LAG, nper,
                    lambda c, cr: v_batch(
                        m, c, cr, lambda t: issue(k_hbm, a + 1, c + LAG - nper, t)),
                    carry)
            l, acc = carry
            rows = pl.ds(pl.multiple_of(a * G, G), G)
            out_sc[rows, :] = acc / jnp.sum(l, axis=-1, keepdims=True)

        def group_body(a, carry):
            group(a, False)
            return carry

        lax.fori_loop(0, A - 1, group_body, 0)
        group(A - 1, True)
        o_ref[...] = out_sc[...].astype(o_ref.dtype)

    out = pl.pallas_call(
        kernel,
        in_specs=[pl.BlockSpec(memory_space=pl.ANY)] * 3,
        out_specs=pl.BlockSpec(memory_space=pltpu.VMEM),
        out_shape=jax.ShapeDtypeStruct((BH, D), q.dtype),
        scratch_shapes=[
            pltpu.VMEM((A, G, D), q.dtype),
            pltpu.VMEM((NB, NS, T, TR, D), k.dtype),
            pltpu.SemaphoreType.DMA((1,)),
            pltpu.SemaphoreType.DMA((NB,)),
            pltpu.SemaphoreType.DMA((len(PARTS),)),
            pltpu.VMEM((U, nper, G, R), jnp.float32),
            pltpu.VMEM((BH, D), jnp.float32),
        ],
        compiler_params=_compiler_params(),
    )(q3, k5, v5)
    return out.reshape(B, Hq, Sq, D)
```

```python
import jax
import jax.numpy as jnp
import numpy as np
from jax import lax
import jax.experimental.pallas as pl
import jax.experimental.pallas.tpu as pltpu

_G = 8
_U = 4
_R = 128
_TR = 8
_HI_FRAC = 8
_NB = 8
_LAG = 5
_PARTS = (16, 8, 8)


def _compiler_params():
    try:
        return pltpu.CompilerParams(disable_semaphore_checks=True)
    except TypeError:
        return pltpu.CompilerParams()


@jax.jit
def pallas_standalone__gqa_softmax__decode_kernel(
    q: jax.Array,
    k: jax.Array,
    v: jax.Array,
):
    B, Hq, Sq, D = q.shape
    Hkv, Sk = k.shape[1], k.shape[2]
    assert Sq == 1 and Hq == Hkv, "decode shape with one KV head per query head"
    G, U, R, TR, NB, LAG, PARTS = _G, _U, _R, _TR, _NB, _LAG, _PARTS
    BH = B * Hq
    A = BH // G
    NS = G * U
    L = Sk // U
    nper = L // R
    T = R // TR
    assert BH % G == 0 and Sk % (U * R) == 0 and R % D == 0 and NS % T == 0
    assert nper % NB == 0 and LAG < NB and LAG < nper and sum(PARTS) == NS
    part_start = [sum(PARTS[:j]) for j in range(len(PARTS))]
    scale = float(np.asarray(D ** -0.5, dtype=q.dtype))

    def round_to_input_dtype(x):
        return x.astype(q.dtype).astype(jnp.float32)

    q3 = q.reshape(A, G, D)
    k5 = k.reshape(A, NS, L // TR, TR, D)
    v5 = v.reshape(A, NS, L // TR, TR, D)

    def kernel(q_hbm, k_hbm, v_hbm, o_ref,
               qbuf, buf, qsem, sem, last_sem, s_sc, out_sc):
        def start_copies(src, a, c, t, s0, sn, dma_sem):
            n_hi = sn // _HI_FRAC
            for lo, n, prio in ((s0 + sn - n_hi, n_hi, 0), (s0, sn - n_hi, 1)):
                pltpu.make_async_copy(
                    src.at[a, pl.ds(lo, n), pl.ds(c * T + t, 1)],
                    buf.at[c % NB, pl.ds(lo, n), pl.ds(t, 1)],
                    dma_sem,
                ).start(priority=prio)

        def issue(src, a, c, t):
            start_copies(src, a, c, t, 0, NS, sem.at[c % NB])

        def issue_last(src, a, c, t):
            for i in range(t * len(PARTS), (t + 1) * len(PARTS)):
                j, tt = divmod(i, T)
                start_copies(src, a, c, tt, part_start[j], PARTS[j], last_sem.at[j])

        def wait(view, dma_sem):
            pltpu.make_async_copy(view, view, dma_sem).wait()

        q_copy = pltpu.make_async_copy(q_hbm, qbuf, qsem.at[0])
        for j in range(LAG):
            for t in range(T):
                issue(k_hbm, 0, j, t)
            if j == 0:
                q_copy.start()
        q_copy.wait()

        row_d = lax.broadcasted_iota(jnp.int32, (G, D), 0)
        row_r = lax.broadcasted_iota(jnp.int32, (G, R), 0)

        def interleave(tile, order, nxt):
            for t in range(T):
                if nxt is not None:
                    nxt(t)
                for s in order[t * NS // T:(t + 1) * NS // T]:
                    tile(s)

        def k_batch(q8, c, mx, nxt):
            slot = c % NB
            wait(buf.at[slot], sem.at[slot])
            sc = [None] * U

            def tile(s):
                g, u = divmod(s, U)
                sg = lax.dot_general(
                    q8, buf[slot, s].reshape(R, D), (((1,), (1,)), ((), ())),
                    preferred_element_type=jnp.float32)
                sc[u] = sg if g == 0 else jnp.where(row_r == g, sg, sc[u])

            interleave(tile, [g * U + u for u in range(U) for g in range(G)], nxt)
            for u in range(U):
                s = round_to_input_dtype(round_to_input_dtype(sc[u]) * scale)
                s_sc[u, c] = s
                for w in range(R // D):
                    mx = jnp.maximum(mx, s[:, w * D:(w + 1) * D])
            return mx

        def v_batch(m, c, carry, nxt, in_parts=False):
            l, acc = carry
            slot = c % NB
            ps = []
            for u in range(U):
                p = jnp.exp(s_sc[u, c] - m)
                for w in range(R // D):
                    l = l + p[:, w * D:(w + 1) * D]
                ps.append(p.astype(v_hbm.dtype))
            if not in_parts:
                wait(buf.at[slot], sem.at[slot])
            st = {}

            def tile(s):
                g, u = divmod(s, U)
                if in_parts and s in part_start:
                    j = part_start.index(s)
                    wait(buf.at[slot, pl.ds(s, PARTS[j])], last_sem.at[j])
                og = jnp.dot(ps[u], buf[slot, s].reshape(R, D),
                             preferred_element_type=jnp.float32)
                og = og if u == 0 else og + st["head"]
                if u < U - 1:
                    st["head"] = og
                else:
                    st["out"] = og if g == 0 else jnp.where(row_d == g, og, st["out"])

            interleave(tile, list(range(NS)), nxt)
            return l, acc + st["out"]

        def group(a, last):
            q8 = qbuf[a]
            mx = jnp.full((G, D), -jnp.inf, jnp.float32)
            mx = lax.fori_loop(
                0, nper - LAG,
                lambda c, mx: k_batch(
                    q8, c, mx, lambda t: issue(k_hbm, a, c + LAG, t)), mx)
            mx = lax.fori_loop(
                nper - LAG, nper,
                lambda c, mx: k_batch(
                    q8, c, mx, lambda t: issue(v_hbm, a, c + LAG - nper, t)), mx)
            m = jnp.max(mx, axis=-1, keepdims=True)
            carry = (jnp.zeros((G, D), jnp.float32), jnp.zeros((G, D), jnp.float32))
            carry = lax.fori_loop(
                0, nper - LAG - (1 if last else 0),
                lambda c, cr: v_batch(
                    m, c, cr, lambda t: issue(v_hbm, a, c + LAG, t)), carry)
            if last:
                carry = v_batch(m, nper - LAG - 1, carry,
                                lambda t: issue_last(v_hbm, a, nper - 1, t))
                carry = lax.fori_loop(
                    nper - LAG, nper - 1,
                    lambda c, cr: v_batch(m, c, cr, None), carry)
                carry = v_batch(m, nper - 1, carry, None, in_parts=True)
            else:
                carry = lax.fori_loop(
                    nper - LAG, nper,
                    lambda c, cr: v_batch(
                        m, c, cr, lambda t: issue(k_hbm, a + 1, c + LAG - nper, t)),
                    carry)
            l, acc = carry
            rows = pl.ds(pl.multiple_of(a * G, G), G)
            out_sc[rows, :] = acc / jnp.sum(l, axis=-1, keepdims=True)

        def group_body(a, carry):
            group(a, False)
            return carry

        lax.fori_loop(0, A - 1, group_body, 0)
        group(A - 1, True)
        o_ref[...] = out_sc[...].astype(o_ref.dtype)

    out = pl.pallas_call(
        kernel,
        in_specs=[pl.BlockSpec(memory_space=pl.ANY)] * 3,
        out_specs=pl.BlockSpec(memory_space=pltpu.VMEM),
        out_shape=jax.ShapeDtypeStruct((BH, D), q.dtype),
        scratch_shapes=[
            pltpu.VMEM((A, G, D), q.dtype),
            pltpu.VMEM((NB, NS, T, TR, D), k.dtype),
            pltpu.SemaphoreType.DMA((1,)),
            pltpu.SemaphoreType.DMA((NB,)),
            pltpu.SemaphoreType.DMA((len(PARTS),)),
            pltpu.VMEM((U, nper, G, R), jnp.float32),
            pltpu.VMEM((BH, D), jnp.float32),
        ],
        compiler_params=_compiler_params(),
    )(q3, k5, v5)
    return out.reshape(B, Hq, Sq, D)
```

```python
import jax
import jax.numpy as jnp
import numpy as np
from jax import lax
import jax.experimental.pallas as pl
import jax.experimental.pallas.tpu as pltpu

_G = 8
_U = 4
_R = 128
_TR = 8
_HI_FRAC = 8
_NB = 8
_LAG = 5
_PARTS = (16, 8, 8)


def _compiler_params():
    vmem = 48 * 1024 * 1024
    try:
        return pltpu.CompilerParams(
            vmem_limit_bytes=vmem, disable_semaphore_checks=True)
    except TypeError:
        return pltpu.CompilerParams(vmem_limit_bytes=vmem)


@jax.jit
def pallas_standalone__gqa_softmax__decode_kernel(
    q: jax.Array,
    k: jax.Array,
    v: jax.Array,
):
    B, Hq, Sq, D = q.shape
    Hkv, Sk = k.shape[1], k.shape[2]
    assert Sq == 1 and Hq == Hkv, "decode shape with one KV head per query head"
    G, U, R, TR, NB, LAG, PARTS = _G, _U, _R, _TR, _NB, _LAG, _PARTS
    BH = B * Hq
    A = BH // G
    NS = G * U
    L = Sk // U
    nper = L // R
    T = R // TR
    assert BH % G == 0 and Sk % (U * R) == 0 and R % D == 0 and NS % T == 0
    assert NB & (NB - 1) == 0 and nper % NB == 0 and LAG < NB and LAG < nper
    assert sum(PARTS) == NS
    part_start = [sum(PARTS[:j]) for j in range(len(PARTS))]
    dtype = q.dtype
    assert k.dtype == dtype and v.dtype == dtype
    scale = float(np.asarray(D ** -0.5, dtype=dtype))

    def round_to_input_dtype(x):
        return x.astype(dtype).astype(jnp.float32)

    q3 = q.reshape(A, G, D)
    k5 = k.reshape(A, NS, L // TR, TR, D)
    v5 = v.reshape(A, NS, L // TR, TR, D)

    def kernel(q_hbm, k_hbm, v_hbm, o_ref,
               qbuf, buf, qsem, sem, last_sem, s_sc, out_sc):
        def issuer(src, a, c, in_parts=False):
            slot = c & (NB - 1)
            tile0 = c * T

            def start(t, s0, sn, dma_sem):
                n_hi = max(2, sn // _HI_FRAC)
                src_tile = pl.ds(tile0 + t, 1)
                for lo, n, prio in ((s0, n_hi, 0), (s0 + n_hi, sn - n_hi, 1)):
                    pltpu.make_async_copy(
                        src.at[a, pl.ds(lo, n), src_tile],
                        buf.at[slot, pl.ds(lo, n), pl.ds(t, 1)],
                        dma_sem,
                    ).start(priority=prio)

            def step(t):
                if not in_parts:
                    start(t, 0, NS, sem.at[slot])
                    return
                for i in range(t * len(PARTS), (t + 1) * len(PARTS)):
                    j, tt = divmod(i, T)
                    start(tt, part_start[j], PARTS[j], last_sem.at[j])

            return step

        def wait(view, dma_sem):
            pltpu.make_async_copy(view, view, dma_sem).wait()

        q_copy = pltpu.make_async_copy(q_hbm, qbuf, qsem.at[0])
        for j in range(LAG):
            step = issuer(k_hbm, 0, j)
            for t in range(T):
                step(t)
            if j == 0:
                q_copy.start()
        q_copy.wait()

        row_d = lax.broadcasted_iota(jnp.int32, (G, D), 0)
        row_r = lax.broadcasted_iota(jnp.int32, (G, R), 0)

        def interleave(tile, order, nxt):
            for t in range(T):
                if nxt is not None:
                    nxt(t)
                for s in order[t * NS // T:(t + 1) * NS // T]:
                    tile(s)

        def k_batch(q8, c, mx, nxt):
            slot = c & (NB - 1)
            wait(buf.at[slot], sem.at[slot])
            sc = [None] * U

            def tile(s):
                g, u = divmod(s, U)
                sg = lax.dot_general(
                    q8, buf[slot, s].reshape(R, D), (((1,), (1,)), ((), ())),
                    preferred_element_type=jnp.float32)
                sc[u] = sg if g == 0 else jnp.where(row_r == g, sg, sc[u])

            interleave(tile, [g * U + u for u in range(U) for g in range(G)], nxt)
            for u in range(U):
                s = round_to_input_dtype(round_to_input_dtype(sc[u]) * scale)
                s_sc[u, c] = s
                for w in range(R // D):
                    mx = jnp.maximum(mx, s[:, w * D:(w + 1) * D])
            return mx

        def v_batch(m, c, carry, nxt, in_parts=False):
            l, acc = carry
            slot = c & (NB - 1)
            ps = []
            for u in range(U):
                p = jnp.exp(s_sc[u, c] - m)
                for w in range(R // D):
                    l = l + p[:, w * D:(w + 1) * D]
                ps.append(p.astype(dtype))
            if not in_parts:
                wait(buf.at[slot], sem.at[slot])
            st = {}

            def tile(s):
                g, u = divmod(s, U)
                if in_parts and s in part_start:
                    j = part_start.index(s)
                    wait(buf.at[slot, pl.ds(s, PARTS[j])], last_sem.at[j])
                og = jnp.dot(ps[u], buf[slot, s].reshape(R, D),
                             preferred_element_type=jnp.float32)
                og = og if u == 0 else og + st["head"]
                if u < U - 1:
                    st["head"] = og
                else:
                    st["out"] = og if g == 0 else jnp.where(row_d == g, og, st["out"])

            interleave(tile, list(range(NS)), nxt)
            return l, acc + st["out"]

        def group(a, last):
            q8 = qbuf[a]
            mx = jnp.full((G, D), -jnp.inf, jnp.float32)
            mx = lax.fori_loop(
                0, nper - LAG,
                lambda c, mx: k_batch(q8, c, mx, issuer(k_hbm, a, c + LAG)), mx)
            mx = lax.fori_loop(
                nper - LAG, nper,
                lambda c, mx: k_batch(q8, c, mx, issuer(v_hbm, a, c + (LAG - nper))),
                mx)
            m = jnp.max(mx, axis=-1, keepdims=True)
            carry = (jnp.zeros((G, D), jnp.float32), jnp.zeros((G, D), jnp.float32))
            carry = lax.fori_loop(
                0, nper - LAG - (1 if last else 0),
                lambda c, cr: v_batch(m, c, cr, issuer(v_hbm, a, c + LAG)), carry)
            if last:
                carry = v_batch(m, nper - LAG - 1, carry,
                                issuer(v_hbm, a, nper - 1, in_parts=True))
                carry = lax.fori_loop(
                    nper - LAG, nper - 1,
                    lambda c, cr: v_batch(m, c, cr, None), carry)
                carry = v_batch(m, nper - 1, carry, None, in_parts=True)
            else:
                carry = lax.fori_loop(
                    nper - LAG, nper,
                    lambda c, cr: v_batch(
                        m, c, cr, issuer(k_hbm, a + 1, c + (LAG - nper))),
                    carry)
            l, acc = carry
            out_sc[a] = acc / jnp.sum(l, axis=-1, keepdims=True)

        def group_body(a, carry):
            group(a, False)
            return carry

        lax.fori_loop(0, A - 1, group_body, 0)
        group(A - 1, True)
        o_ref[...] = out_sc[...].reshape(BH, D).astype(o_ref.dtype)

    out = pl.pallas_call(
        kernel,
        in_specs=[pl.BlockSpec(memory_space=pl.ANY)] * 3,
        out_specs=pl.BlockSpec(memory_space=pltpu.VMEM),
        out_shape=jax.ShapeDtypeStruct((BH, D), dtype),
        scratch_shapes=[
            pltpu.VMEM((A, G, D), dtype),
            pltpu.VMEM((NB, NS, T, TR, D), dtype),
            pltpu.SemaphoreType.DMA((1,)),
            pltpu.SemaphoreType.DMA((NB,)),
            pltpu.SemaphoreType.DMA((len(PARTS),)),
            pltpu.VMEM((U, nper, G, R), jnp.float32),
            pltpu.VMEM((A, G, D), jnp.float32),
        ],
        compiler_params=_compiler_params(),
    )(q3, k5, v5)
    return out.reshape(B, Hq, Sq, D)
```
